```python
import jax
import jax.numpy as jnp

def _softmax(x, axis=-1):
    return jax.nn.softmax(x, axis=axis)

def _gelu(x):
    return jax.nn.gelu(x, approximate=True)

def _silu(x):
    return jax.nn.silu(x)

def _sigmoid(x):
    return jax.nn.sigmoid(x)

def _layernorm(x, axis=-1, eps=1e-05):
    m = jnp.mean(x, axis=axis, keepdims=True)
    v = jnp.var(x, axis=axis, keepdims=True)
    return (x - m) / jnp.sqrt(v + eps)

def _scatter_add(tgt, idx, src, axis=0):
    return tgt.at[idx].add(src)

def _segment_sum(src, seg, n):
    return jax.ops.segment_sum(src, seg, n)

class _Rng:

    def __init__(self, key):
        self._k = key

    def _next(self):
        self._k, sub = jax.random.split(self._k)
        return sub

    def normal(self, shape):
        return jax.random.normal(self._next(), shape, dtype=jnp.bfloat16)

    def randint(self, lo, hi, shape):
        return jax.random.randint(self._next(), shape, lo, hi, dtype=jnp.int32)

    def uniform(self, shape, lo=0.0, hi=1.0):
        return jax.random.uniform(self._next(), shape, jnp.bfloat16, lo, hi)

    def permutation(self, n):
        return jax.random.permutation(self._next(), n)
kernel_name = 'adaLN_cond__memory_aug_infini_attn__dense_activation_gelu__prompt'

def _fwd_setup_inputs():
    _rng = _Rng(jax.random.key(int.from_bytes(__import__("os").urandom(4), "little")))
    _w = lambda a: (lambda t: t.astype(jnp.bfloat16) if jnp.issubdtype(t.dtype, jnp.floating) else t)(jnp.asarray(a))

    def _A_setup():
        B, S, D, H = (1, 2048, 640, 32)
        N = 4
        L = max(1, S // N)
        sc = D ** (-0.5)
        return {'x': _w((lambda *s: _rng.normal(s) * 0.05)(B, N * L, D)), 'wq': _w((lambda *s: _rng.normal(s) * 0.05)(D, D) * sc), 'wk': _w((lambda *s: _rng.normal(s) * 0.05)(D, D) * sc), 'wv': _w((lambda *s: _rng.normal(s) * 0.05)(D, D) * sc), 'wo': _w((lambda *s: _rng.normal(s) * 0.05)(D, D) * sc), 'beta': _w((lambda *s: _rng.normal(s) * 0.05)(H))}
    _A_in = _A_setup()

    def _B_setup():
        B, S, D, F = (1, 2048, 640, 1728)
        return {'x': _w((lambda *s: _rng.normal(s) * 0.05)(B, S, D)), 'w1': _w((lambda *s: _rng.normal(s) * 0.05)(D, F) * D ** (-0.5)), 'b1': _w((lambda *s: _rng.normal(s) * 0.05)(F) * 0.01), 'w2': _w((lambda *s: _rng.normal(s) * 0.05)(F, D) * F ** (-0.5)), 'b2': _w((lambda *s: _rng.normal(s) * 0.05)(D) * 0.01)}
    _B_in = _B_setup()
    return {'A_x': _A_in['x'], 'A_wq': _A_in['wq'], 'A_wk': _A_in['wk'], 'A_wv': _A_in['wv'], 'A_wo': _A_in['wo'], 'A_beta': _A_in['beta'], 'B_x': _B_in['x'], 'B_w1': _B_in['w1'], 'B_b1': _B_in['b1'], 'B_w2': _B_in['w2'], 'B_b2': _B_in['b2'], 'c': _w((lambda *s: _rng.normal(s) * 0.05)(1, 640)), 'w_mod': _w((lambda *s: _rng.normal(s) * 0.05)(640, 6 * 640) * 640 ** (-0.5))}

def _fwd_reference(A_x, A_wq, A_wk, A_wv, A_wo, A_beta, B_x, B_w1, B_b1, B_w2, B_b2, c, w_mod):

    def _A_ref(x, wq, wk, wv, wo, beta):
        B, S, D = x.shape
        H = 32
        Dh = D // H
        N = 4
        L = S // N
        q = (lambda x, *d: x.transpose(*d))((x @ wq).reshape(B, S, H, Dh), 0, 2, 1, 3).reshape(B, H, N, L, Dh)
        k = (lambda x, *d: x.transpose(*d))((x @ wk).reshape(B, S, H, Dh), 0, 2, 1, 3).reshape(B, H, N, L, Dh)
        v = (lambda x, *d: x.transpose(*d))((x @ wv).reshape(B, S, H, Dh), 0, 2, 1, 3).reshape(B, H, N, L, Dh)
        phi = lambda t: jnp.where(t > 0, t + 1.0, jnp.exp(t))
        scale = Dh ** (-0.5)
        ar = jnp.arange(L)
        mask = (lambda x, dt: x.astype(dt))(ar[:, None] < ar[None, :], x.dtype) * -1000000000.0
        g = _sigmoid(beta).reshape(1, H, 1, 1)
        M = jnp.einsum('bhd,bhe->bhde', q[:, :, 0, 0, :] * 0.0, q[:, :, 0, 0, :] * 0.0)
        z = q[:, :, 0, 0, :] * 0.0
        outs = []
        for s in range(N):
            qs, ks, vs = (q[:, :, s].copy(), k[:, :, s].copy(), v[:, :, s].copy())
            logits = jnp.einsum('bhqd,bhkd->bhqk', qs, ks) * scale + mask
            p = _softmax(logits, axis=-1)
            a_dot = jnp.einsum('bhqk,bhkd->bhqd', p, vs)
            pq = phi(qs)
            num = jnp.einsum('bhld,bhde->bhle', pq, M)
            den = jnp.einsum('bhld,bhd->bhl', pq, z)[..., None] + 1e-06
            a_mem = num / den
            o = g * a_mem + (1.0 - g) * a_dot
            outs.append(o)
            pk = phi(ks)
            M = M + jnp.einsum('bhld,bhle->bhde', pk, vs)
            z = z + jnp.einsum('bhld->bhd', pk)
        o = (lambda x, *d: x.transpose(*d))(jnp.stack(outs, 2).reshape(B, H, S, Dh), 0, 2, 1, 3).reshape(B, S, D)
        return o @ wo

    def _B_ref(x, w1, b1, w2, b2):
        h = jnp.einsum('bsd,df->bsf', x, w1) + b1
        h = _gelu(h)
        return jnp.einsum('bsf,fd->bsd', h, w2) + b2
    x = A_x
    mod = (_silu(c) @ w_mod).reshape(c.shape[0], 6, 1, -1)
    sa, ca, ga, sb, cb, gb = (mod[:, 0].copy(), mod[:, 1].copy(), mod[:, 2].copy(), mod[:, 3].copy(), mod[:, 4].copy(), mod[:, 5].copy())
    h = _layernorm(x, axis=-1) * (1 + ca) + sa
    x = x + ga * _A_ref(h, A_wq, A_wk, A_wv, A_wo, A_beta)
    h = _layernorm(x, axis=-1) * (1 + cb) + sb
    x = x + gb * _B_ref(h, B_w1, B_b1, B_w2, B_b2)
    return x

def setup_inputs():
    _inp = _fwd_setup_inputs()
    _gk = jax.random.fold_in(jax.random.key(int.from_bytes(__import__("os").urandom(4), "little")), 2 ** 31 - 1)
    _shapes = [[1, 2048, 640]]
    _dtypes = ['bfloat16']
    _gks = jax.random.split(_gk, len(_shapes))
    _gs = [jax.random.normal(k, s, dtype=jnp.dtype(d)) * 0.05 for k, s, d in zip(_gks, _shapes, _dtypes)]
    _inp['grad_out'] = _gs[0]
    return _inp

def reference(A_x, A_wq, A_wk, A_wv, A_wo, A_beta, B_w1, B_b1, B_w2, B_b2, c, w_mod, B_x, grad_out):
    _const = dict(B_x=B_x)

    def _f(*_d):
        return _fwd_reference(**{'A_x': _d[0], 'A_wq': _d[1], 'A_wk': _d[2], 'A_wv': _d[3], 'A_wo': _d[4], 'A_beta': _d[5], 'B_w1': _d[6], 'B_b1': _d[7], 'B_w2': _d[8], 'B_b2': _d[9], 'c': _d[10], 'w_mod': _d[11], **_const})
    _out, _vjp = jax.vjp(_f, A_x, A_wq, A_wk, A_wv, A_wo, A_beta, B_w1, B_b1, B_w2, B_b2, c, w_mod)
    _grads = _vjp(grad_out)
    _out0 = jnp.asarray(_out)
    return (_out0, *[jnp.asarray(_g) for _g in _grads])
```

```python
import math

import jax
import jax.numpy as jnp
from jax import lax
import jax.experimental.pallas as pl
import jax.experimental.pallas.tpu as pltpu

S, D, H, DH, NSEG, F = 2048, 640, 32, 20, 4, 1728
L = S // NSEG
HG = 4
G = H // HG
GR = HG * DH
QB = 128
HB = QB // 2
NJ = L // QB
MR = GR + 16
GUF = 8
GUB = 8
NSLOT = 8
RC = 128
NC = L // RC
NZ = 8
FSPLIT = (0, 256, 768, F)
LAGS = (5, 6, 3)
CHAIN = 3
FCHAIN = 1
USPLIT = (0, 256, 512, 768, 1024, 1280, 1536, F)
FK = 512
FP = 3
DC = 16
EP = 10
LN1P = ((9, 5, 14, 8), (2, 9, 12, 9))
WSPLIT = (0, 192, 896, F)
BORDER = [(i, j) for i in range(4) for j in range(i, 4)]
LAG_B, LAG_C, LAG_Q = LAGS
EPS = 1e-5
SCALE = DH ** -0.5
LOG2E = math.log2(math.e)
GC0 = math.sqrt(2.0 / math.pi)
GC1 = 0.044715
BF = jnp.bfloat16
F32 = jnp.float32

_NN = (((1,), (0,)), ((), ()))
_NT = (((1,), (1,)), ((), ()))
_TN = (((0,), (0,)), ((), ()))


def _dot(a, b, dims=_NN):
    return lax.dot_general(a, b, dims, preferred_element_type=F32)


def _phi(t):
    return jnp.where(t > 0, t + 1.0, jnp.exp(t))


U32 = jnp.uint32
ONES2 = 0x3F803F80


def _pk(x):
    return pltpu.bitcast(x, U32)


def _upk(x):
    return pltpu.bitcast(x, BF)


def _ipk(a, b):
    return pltpu.pack_elementwise([a, b], packed_dtype=BF)


def _iupk(x, idx):
    return pltpu.unpack_elementwise(x, index=idx, packed_dtype=BF, unpacked_dtype=F32)


def _tri(i, j):
    return j * (j + 1) // 2 + i


def _pairs(x):
    n, m = x.shape
    x4 = x.reshape(n // 16, 2, 8, m)
    return x4[:, 0].reshape(n // 2, m), x4[:, 1].reshape(n // 2, m)


def _deint(xt):
    nat = _pk(xt.T)
    ev = _iupk(nat, 0).reshape(L // 16, 1, 8, 128)
    od = _iupk(nat, 1).reshape(L // 16, 1, 8, 128)
    return _pk(jnp.concatenate([ev, od], axis=1).reshape(L, 128).astype(BF))


def _assemble(r):
    n = r[0].shape[1]
    lo = lax.broadcasted_iota(jnp.int32, (8, n), 0) < 4
    return jnp.concatenate([
        r[0][0:16],
        jnp.where(lo, r[0][16:24], r[1][0:8]),
        r[1][8:24],
        r[2][8:24],
        jnp.where(lo, r[2][24:32], r[3][8:16]),
        r[3][16:32],
    ], axis=0)


def _expand(r):
    n = r.shape[1]
    b = [jnp.broadcast_to(r[h:h + 1], (8, n)) for h in range(HG)]
    lo = lax.broadcasted_iota(jnp.int32, (8, n), 0) < 4
    return jnp.concatenate([b[0], b[0], jnp.where(lo, b[0], b[1]), b[1], b[1],
                            b[2], b[2], jnp.where(lo, b[2], b[3]), b[3], b[3]], axis=0)


def _segsum(t):
    n = t.shape[1]
    lo = lax.broadcasted_iota(jnp.int32, (8, n), 0) < 4
    v = [t[8 * r:8 * r + 8] for r in range(10)]
    parts = [v[0] + v[1] + jnp.where(lo, v[2], 0.0), v[3] + v[4] + jnp.where(lo, 0.0, v[2]),
             v[5] + v[6] + jnp.where(lo, v[7], 0.0), v[8] + v[9] + jnp.where(lo, 0.0, v[7])]
    return [jnp.sum(q, axis=0, keepdims=True) for q in parts]


def _kernel(x_hbm, go_hbm, wq_hbm, wk_hbm, wv_hbm, wo_hbm, w1T_hbm, w2_hbm, wm_hbm,
            beta_hbm, b1_hbm, b2_hbm, c_hbm,
            out_hbm, dx_hbm, dwq_hbm, dwk_hbm, dwv_hbm, dwo_hbm, dbeta_hbm,
            dw1T_hbm, db1_hbm, dw2_hbm, db2_hbm, dc_hbm, dwm_hbm,
            beta_v, b1_v, b2_v, c_v, b1r_v, b2r_v,
            x_v, go_v, wqkv_v, wqkvT_v, wo_v, w1T_v, w2_v, wm_v,
            mod_v, gate_v, h1T_v, qkvT_v, kvn_v, mem_v, dmem_v,
            pT_v, adot_v, amem_v, linv_v, dinv_v, oT_v, doT_v, dqkvT_v,
            out_v,
            dwo_acc, dw1T_acc, dw2_acc, silb_v, dg_acc,
            dwm_o, wT_v, db1_acc,
            zv_v, zo_s, zs_s, isem, osem, *bufs):
    st_v = bufs[0:NSLOT]
    ybuf, dx2buf, x2buf = (bufs[NSLOT + k * NC:NSLOT + (k + 1) * NC] for k in range(3))
    cps = [
        pltpu.make_async_copy(x_hbm.at[0:L, :], x_v.at[0:L, :], isem.at[0]),
        pltpu.make_async_copy(wm_hbm.at[:, 0:2 * D], wm_v.at[:, 0:2 * D], isem.at[1]),
        pltpu.make_async_copy(wq_hbm, wqkv_v.at[:, 0:D], isem.at[2]),
        pltpu.make_async_copy(wk_hbm, wqkv_v.at[:, D:2 * D], isem.at[3]),
        pltpu.make_async_copy(wv_hbm, wqkv_v.at[:, 2 * D:3 * D], isem.at[4]),
        pltpu.make_async_copy(x_hbm.at[L:2 * L, :], x_v.at[L:2 * L, :], isem.at[5]),
        pltpu.make_async_copy(wm_hbm.at[:, 2 * D:6 * D], wm_v.at[:, 2 * D:6 * D], isem.at[6]),
        pltpu.make_async_copy(wo_hbm, wo_v, isem.at[7]),
        pltpu.make_async_copy(w1T_hbm, w1T_v, isem.at[8]),
        pltpu.make_async_copy(w2_hbm, w2_v, isem.at[9]),
    ] + [pltpu.make_async_copy(go_hbm.at[s * L:(s + 1) * L, :], go_v.at[s * L:(s + 1) * L, :],
                               isem.at[13 - s]) for s in range(NSEG - 1, -1, -1)]
    cps.append(pltpu.make_async_copy(x_hbm.at[2 * L:S, :], x_v.at[2 * L:S, :], isem.at[14]))
    small = [pltpu.make_async_copy(a, b, isem.at[16 + k]) for k, (a, b) in enumerate(
        ((c_hbm, c_v), (beta_hbm, beta_v), (b1_hbm, b1_v), (b2_hbm, b2_v)))]
    for cp in small:
        cp.start()
    for i in (1, 0, 3, 4, 2, 5):
        cps[i].start()
    zv_v[...] = jnp.zeros((8, 128), jnp.int32)
    zcp = pltpu.make_async_copy(zv_v, zo_s, isem.at[15])
    zcp.start()
    for k in range(NZ):
        zs_s[k] = 0

    for cp in small:
        cp.wait()
    b1w = jnp.broadcast_to(b1_v[...].astype(F32).reshape(1, F), (128, F))
    b1r_v[0:F - 64, :] = b1w[:, 0:F - 64].T
    b1r_v[F - 64:F, :] = b1w[:, F - 128:F].T[64:128]
    b2r_v[...] = b2_v[...].astype(F32).reshape(1, D)
    cf = c_v[...].astype(F32)
    sig_c = jax.nn.sigmoid(cf)
    silu_c = cf * sig_c
    silu16 = jnp.broadcast_to(silu_c, (16, D)).astype(BF)

    head_of_row = lax.broadcasted_iota(jnp.int32, (D, H), 0) // DH
    onehot = head_of_row == lax.broadcasted_iota(jnp.int32, (D, H), 1)
    gate_row = jax.nn.sigmoid(beta_v[...].astype(F32).reshape(1, H))
    gate_col = jnp.sum(jnp.where(onehot, gate_row, 0.0), axis=1, keepdims=True)
    gate_v[...] = jnp.broadcast_to(gate_col, (D, 128)).reshape(G, GR, 128)

    silb_v[...] = jnp.broadcast_to(silu_c.astype(BF).astype(F32), (128, D)).T

    bd_r = lax.broadcasted_iota(jnp.int32, (MR, GR), 0)
    bd_c = lax.broadcasted_iota(jnp.int32, (MR, GR), 1) // DH
    bd_mask = jnp.where(bd_r < GR, bd_r // DH, bd_r - GR) == bd_c
    pr = lax.broadcasted_iota(jnp.int32, (128 - GR, L), 0)

    zcp.wait()
    ztrue = zo_s[0, 0] == 0
    zz = [zs_s[k] for k in range(NZ)]

    def put(buf, val, r0=0):
        buf[pl.ds(pl.multiple_of(zz[0] + r0, 8), RC), :] = val

    def get(buf, k, r0=0):
        return buf[pl.ds(pl.multiple_of(zz[k] + r0, 8), RC), :]

    def getb(ref, r0, k):
        return ref[pl.ds(pl.multiple_of(r0 + zz[k], 16), RC), :].astype(F32)

    def rmean(t):
        return jnp.broadcast_to(jnp.mean(t, axis=1, keepdims=True), (t.shape[0], 128))

    def wide(m):
        return jnp.concatenate([m] * (D // 128), axis=1)

    def toks(res, k0, n, ntot):
        m, out = res.shape[0], []
        for k in range(k0, k0 + n):
            pos = k * (m * (D // 128) // 8) // ntot
            r, c = pos % (m // 8) * 8, pos // (m // 8) * 128
            out.append(res[r:r + 8, c:c + 128])
        return jnp.concatenate(out, axis=0)

    def pace(v, tok):
        if tok is None:
            return v
        if tok.shape[0] != v.shape[0]:
            tok = jnp.concatenate([tok] * (v.shape[0] // tok.shape[0]), axis=0)
        return jnp.where(ztrue, v, tok)

    mu1, rs1, h1c = {}, {}, {}

    def ln1_mean(s):
        for c in range(NC):
            mu1[s, c] = rmean(getb(x_v, s * L + c * RC, 4))

    def ln1_rstd(s, c, tok=None):
        xc = getb(x_v, s * L + c * RC, 5) - wide(pace(mu1[s, c], tok))
        rs1[s, c] = lax.rsqrt(rmean(xc * xc) + EPS)

    def ln1_mod(s, c, tok=None):
        xh = (getb(x_v, s * L + c * RC, 6) - wide(pace(mu1[s, c], tok))) * wide(rs1[s, c])
        h1c[s, c] = (xh * (1.0 + mod_v[0:1, D:2 * D]) + mod_v[0:1, 0:D]).astype(BF)
        h1T_v[s, :, c * RC:(c + 1) * RC] = _pk(h1c[s, c].T)

    def w_t(i):
        wT_v[i] = _pk(wqkv_v[:, i * D:(i + 1) * D].T).reshape(G, GR // 2, D)

    vac, dfp = {}, {}

    def vacc(key, t):
        r = jnp.sum(t.reshape(t.shape[0] // 8, 8, t.shape[1]), axis=0)
        vac[key] = r if key not in vac else vac[key] + r

    def df_rows(s, k, tok):
        gb = jnp.broadcast_to(mod_v[0:1, 5 * D:6 * D], (8, D))
        gb = jnp.concatenate([jnp.where(ztrue, gb, wide(tok))] * 4, axis=0)
        df = go_v[s * L + 32 * k:s * L + 32 * (k + 1), :].astype(F32) * gb
        vacc('b2', df)
        dfp.setdefault(s, []).append(_pk(df.astype(BF)))

    def mem_read(s, g, qb):
        nd = _dot(mem_v[s - 1, g], _phi(qb.astype(F32)).astype(BF))
        dinv = _expand(1.0 / (nd[GR:GR + 8] + 1e-6))
        amem_v[g] = nd[0:GR] * dinv
        dinv_v[g] = dinv

    ones16 = jnp.ones((16, L), BF)
    kpad = jnp.zeros((128 - GR, L), BF)
    vpad = jnp.where(pr < 2, 1.0, 0.0).astype(BF)
    cps[1].wait()
    mod_v[:, 0:2 * D] = _dot(silu16, wm_v[:, 0:2 * D])[0:8]
    cps[0].wait()
    ln1_mean(0)
    for c in range(NC):
        ln1_rstd(0, c)
    for c in range(NC):
        ln1_mod(0, c)
    cps[3].wait()
    w_t(1)
    macc = [None] * G
    for s in range(NSEG):
        tt, tfs = {}, []
        h1 = jnp.concatenate([h1c[s, c] for c in range(NC)], axis=0)
        for n, i in enumerate((1, 2, 0)):
            if s == 0 and n == 1:
                for k in (14,) + tuple(range(6, 14)):
                    cps[k].start()
                for k in (4, 2, 5):
                    cps[k].wait()
                w_t(2)
                w_t(0)
            if s + 1 < NSEG and n == (1 if s == 0 else 0):
                ln1_mean(s + 1)
            for g in range(G):
                tf = _dot(_upk(wT_v[i, g]), h1, _NT)
                tt[i, g] = tf.astype(BF)
                qkvT_v[s, i * G + g] = _pk(tt[i, g])
                tok = tf[0:8, 0:128]
                k = n * G + g
                if i > 0:
                    kvn_v[s, (i - 1) * G + g] = _deint(
                        jnp.concatenate([tt[i, g], kpad if i == 1 else vpad], axis=0))
                else:
                    qs = (tt[i, g].astype(F32) * (SCALE * LOG2E)).astype(BF)
                    qkvT_v[s, 3 * G + g] = _pk(qs)
                    if s + 1 < NSEG:
                        pk = _phi(tt[1, g].astype(F32)).astype(BF)
                        va = jnp.concatenate([tt[2, g], ones16], axis=0)
                        inc = jnp.where(bd_mask, _dot(va, pk, _NT), 0.0)
                        macc[g] = inc if s == 0 else macc[g] + inc
                        mem_v[s, g] = macc[g].astype(BF)
                    else:
                        if g > 0:
                            mem_read(s, g - 1, tt[i, g - 1])
                        if g == G - 1:
                            mem_read(s, g, tt[i, g])
                tfs.append(tf)
                if s == NSEG - 1 and k < L // 32:
                    df_rows(s, k, tok)
                if s == NSEG - 2 and k % 4 == 1 and k // 4 < 5:
                    ms_ = slice(2 * D + k // 4 * 512, 2 * D + (k // 4 + 1) * 512)
                    mod_v[:, ms_] = _dot(silu16, wm_v[:, ms_])[0:8]
        if s + 1 < NSEG:
            def tk(k0, span, c):
                pos = [(c * 16 + q) * span * 10 // 64 for q in range(16)]
                return jnp.concatenate(
                    [tfs[k0 + p // 10][p % 10 * 8:p % 10 * 8 + 8, q % 4 * 128:q % 4 * 128 + 128]
                     for q, p in enumerate(pos)], axis=0)
            k0, n0, k1, n1 = LN1P[min(s, 1)]
            for c in range(NC):
                ln1_rstd(s + 1, c, tk(k0, n0, c))
            for c in range(NC):
                ln1_mod(s + 1, c, tk(k1, n1, c))
        if s == 0:
            cps[14].wait()
        if s == NSEG - 3:
            cps[6].wait()
        if s == NSEG - 2:
            for i in range(7, 11):
                cps[i].wait()
        if s == NSEG - 1:
            cps[11].wait()

    fin = []

    def emit(src, dst, k):
        cp = pltpu.make_async_copy(src, dst, osem.at[k])
        cp.start()
        fin.append(cp)

    prow40 = lax.broadcasted_iota(jnp.int32, (GR // 2, QB), 0) // (DH // 2)
    prow16 = lax.broadcasted_iota(jnp.int32, (16, L), 0)
    crow = lax.broadcasted_iota(jnp.int32, (QB, QB), 0)
    ckey = (crow // 16) * 16 + (crow % 8) * 2 + (crow % 16) // 8
    cbias = jnp.where(ckey > lax.broadcasted_iota(jnp.int32, (QB, QB), 1), -1e30, 0.0)

    lo40 = lax.broadcasted_iota(jnp.int32, (GR // 2, QB), 1) < HB
    lo8 = lax.broadcasted_iota(jnp.int32, (8, QB), 1) < HB
    cbias2 = jnp.where(ckey[0:HB] > lax.broadcasted_iota(jnp.int32, (HB, QB), 1) % HB, -1e30, 0.0)

    def out_copy(s):
        return pltpu.make_async_copy(out_v.at[s * L:(s + 1) * L, :], out_hbm.at[s * L:(s + 1) * L, :],
                                     osem.at[8 + s])

    def dx_copy(s):
        return pltpu.make_async_copy(go_v.at[s * L:(s + 1) * L, :], dx_hbm.at[s * L:(s + 1) * L, :],
                                     osem.at[12 + s])

    def phase2(it, carry):
        s = NSEG - 1 - it
        rows = slice(s * L, (s + 1) * L)
        za, zb = zz[0], zz[1]
        sd = s + zz[2]

        ca = mod_v[0:1, D:2 * D]
        ga, sb = mod_v[0:1, 2 * D:3 * D], mod_v[0:1, 3 * D:4 * D]
        cb, gb = mod_v[0:1, 4 * D:5 * D], mod_v[0:1, 5 * D:6 * D]
        dfb = _upk(jnp.concatenate(dfp.pop(s), axis=0))

        def wacc(acc, stage, idx, val):
            if it == 0:
                acc[idx] = val
            elif it < NSEG - 1:
                acc[idx] += val
            else:
                stage[idx] = (acc[idx] + val).astype(BF)

        das = []

        def da_part(k):
            das.append(_dot(w2_v[FSPLIT[k]:FSPLIT[k + 1], :], dfb, _NT))

        def attn_fwd(gi, c2):
            zq = jnp.zeros((64 - GR // 2, HG * QB), U32)
            steps = [(u, j, i) for u in range(GUF) for j in range(NJ - 1, -1, -1) for i in range(j + 1)]
            va, rq, m8, mx, pp, acc = {}, {}, {}, {}, {}, {}
            atok, ptok, ctok, rq2 = {}, {}, {}, {}

            def gidx(u):
                return u if GUF == G else gi * GUF + u

            def q_tiles(u, j):
                qp = qkvT_v[sd, 3 * G + gidx(u), :, j * QB:(j + 1) * QB]
                top = [jnp.where(prow40 == h, qp, jnp.uint32(0)) for h in range(HG)]
                rq[u, j] = _upk(jnp.concatenate([jnp.concatenate(top, axis=1), zq], axis=0))
                qr = pltpu.roll(qp, HB, 1)
                rq2[u, j] = [_upk(jnp.concatenate(
                    [jnp.where(lo40, jnp.where(prow40 == 2 * p, qr, jnp.uint32(0)), top[2 * p + 1]),
                     zq[:, 0:QB]], axis=0)) for p in range(HG // 2)]
                return [top[h][8 * h:8 * h + 8] | top[h][8 * h + 8:8 * h + 16] for h in range(HG)]

            def a_step(t):
                u, j, i = steps[t]
                g = gidx(u)
                if t == 0:
                    q_tiles(u, j)
                qt = q_tiles(*steps[t + 1][0:2]) if t + 1 < len(steps) and steps[t + 1][2] == 0 else None
                kp = kvn_v[sd, g, i * (QB // 2):(i + 1) * (QB // 2), :]
                if FCHAIN and t - LAG_C - 2 >= 0:
                    ct = ctok[t - LAG_C - 2]
                    if qt is not None:
                        ct = [x | y for x, y in zip(ct, qt)]
                    tok = jnp.concatenate(ptok[t - LAG_C] + ct, axis=0)
                    kp = jnp.where(ztrue, kp, tok)
                if i < j:
                    st = _dot(_upk(kp), rq[u, j])
                    st_v[t % NSLOT][za] = st
                    cm = jnp.max(st.reshape(QB // 8, 8, HG * QB), axis=0)
                else:
                    st = _dot(_upk(kp[0:HB // 2]), rq[u, j])
                    sm = st + jnp.concatenate([cbias[0:HB]] * HG, axis=1)
                    st_v[t % NSLOT][za, 0:HB, :] = sm
                    cm = jnp.max(sm.reshape(HB // 8, 8, HG * QB), axis=0)
                    cm2 = []
                    for p in range(HG // 2):
                        s2 = jnp.concatenate(
                            [_dot(_upk(kp[HB // 2 + r * 16:HB // 2 + (r + 1) * 16]), rq2[u, j][p])
                             for r in range(2)], axis=0) + cbias2
                        st_v[t % NSLOT][za, HB:QB, p * QB:(p + 1) * QB] = s2
                        c2_ = jnp.max(s2.reshape(HB // 8, 8, QB), axis=0)
                        cm2 += [jnp.where(lo8, -jnp.inf, pltpu.roll(c2_, HB, 1)), jnp.where(lo8, -jnp.inf, c2_)]
                    cm = jnp.maximum(cm, jnp.concatenate(cm2, axis=1))
                atok[t] = [pltpu.bitcast(st[0:8, h * QB:(h + 1) * QB], U32) for h in range(HG)]
                m8[u, j] = cm if i == 0 else jnp.maximum(m8[u, j], cm)

            def b_step(t):
                u, j, i = steps[t]
                g = gidx(u)
                if i == 0:
                    mx[u, j] = jnp.max(m8[u, j], axis=0, keepdims=True)
                ps = []
                ptok[t] = []
                for h in range(HG):
                    hs = slice(h * QB, (h + 1) * QB)
                    if i < j:
                        ph = _ipk(*_pairs(jnp.exp2(st_v[t % NSLOT][zb, :, hs] - mx[u, j][:, hs])))
                    else:
                        if h % 2 == 0:
                            m2 = jnp.broadcast_to(mx[u, j][:, h * QB:(h + 2) * QB], (8, 2 * QB))
                            m2 = jnp.where(lo8, pltpu.roll(m2[:, 0:QB], HB, 1), m2[:, QB:2 * QB])[0:1]
                            p2 = st_v[t % NSLOT][zb, HB:QB, h // 2 * QB:(h // 2 + 1) * QB]
                            p2 = _ipk(*_pairs(jnp.exp2(p2 - m2)))
                        ph = _ipk(*_pairs(jnp.exp2(st_v[t % NSLOT][zb, 0:HB, hs] - mx[u, j][:, hs])))
                        hi = pltpu.roll(p2, HB, 1) if h % 2 == 0 else p2
                        ph = jnp.concatenate([ph, jnp.where(lo40[0:32], jnp.uint32(0), hi)], axis=0)
                    pT_v[g, _tri(i, j), :, hs] = ph
                    ps.append(_upk(ph))
                    ptok[t].append(ph[56:64])
                pp[t] = ps

            def c_step(t):
                u, j, i = steps[t]
                g = gidx(u)
                if j == NJ - 1 and i == 0:
                    vp = qkvT_v[sd, 2 * G + g]
                    va[u] = []
                    for h in range(HG):
                        valid = (prow16 >= 2 * h) & (prow16 < 2 * h + DH // 2)
                        va[u].append(jnp.where(valid, vp[8 * h:8 * h + 16], jnp.uint32(ONES2)))
                ps = pp.pop(t)
                r = []
                for h in range(HG):
                    vw = va[u][h][:, i * QB:(i + 1) * QB]
                    if FCHAIN and t + LAG_C - 1 in atok:
                        vw = jnp.concatenate([jnp.where(ztrue, vw[0:8], atok[t + LAG_C - 1][h]), vw[8:16]], axis=0)
                    r.append(_dot(_upk(vw), ps[h]))
                ctok[t] = [pltpu.bitcast(x[0:8], U32) for x in r]
                acc[u, j] = r if i == 0 else [x + y for x, y in zip(acc[u, j], r)]
                if i == j:
                    rs, ls = [], []
                    for h in range(HG):
                        ah = acc[u, j][h]
                        lrow = ah[24:32] if h < 2 else ah[0:8]
                        linv = jnp.concatenate([1.0 / lrow] * 4, axis=0)
                        rs.append(ah * linv)
                        ls.append(linv)
                    js = slice(j * QB, (j + 1) * QB)
                    ad = _assemble(rs)
                    adot_v[g, :, js] = ad
                    linv_v[g, :, js] = _assemble(ls)
                    o = (1.0 - gate_v[g]) * ad
                    if s > 0:
                        o = gate_v[g] * amem_v[g, :, js] + o
                    oT_v[g, :, js] = _pk(o.astype(BF))

            n = len(steps)
            for t in range(n + LAG_C):
                if t < n:
                    a_step(t)
                if t == n - 1:
                    da_part(0)
                if LAG_C > LAG_B and 0 <= t - LAG_C < n:
                    c_step(t - LAG_C)
                if 0 <= t - LAG_B < n:
                    b_step(t - LAG_B)
                if LAG_C == LAG_B and 0 <= t - LAG_C < n:
                    c_step(t - LAG_C)
            return c2

        attn_fwd(0, 0)
        da_part(1)

        oT = _upk(oT_v[...].reshape(D // 2, L))
        y = _dot(oT, wo_v[...], _TN)
        da_part(2)
        mu2, rs2, h2 = [], [], []
        for c in range(NC):
            yc = y[c * RC:(c + 1) * RC]
            put(ybuf[c], yc)
            x2 = getb(x_v, s * L + c * RC, 1) + ga * yc
            put(x2buf[c], x2)
            mu2.append(rmean(x2))
        for c in range(NC):
            xc = get(x2buf[c], 1) - wide(mu2[c])
            rs2.append(lax.rsqrt(rmean(xc * xc) + EPS))
        for c in range(NC):
            xh = (get(x2buf[c], 2) - wide(mu2[c])) * wide(rs2[c])
            h2.append((xh * (1.0 + cb) + sb).astype(BF))
        h2 = jnp.concatenate(h2, axis=0)
        u = jnp.concatenate([_dot(w1T_v[USPLIT[k]:USPLIT[k + 1], :], h2, _NT)
                             for k in range(len(USPLIT) - 1)], axis=0)
        u = u + jnp.concatenate([b1r_v[...]] * (L // 128), axis=1)
        u2 = u * u
        th = jnp.tanh(GC0 * u * (1.0 + GC1 * u2))
        hp = 0.5 * (1.0 + th)
        a = (u * hp).astype(BF)
        fps = [_dot(a[k:k + FK], w2_v[k:min(k + FK, F), :], _TN) for k in range(0, F, FK)]
        f = fps[0] + b2r_v[...]
        for fp in fps[1:]:
            f = f + fp

        for c in range(NC):
            fc = f[c * RC:(c + 1) * RC]
            out_v[s * L + c * RC:s * L + (c + 1) * RC, :] = (get(x2buf[c], 3) + gb * fc).astype(BF)
            vacc(5, getb(go_v, s * L + c * RC, 1) * fc)

        da, du, nd_ = jnp.concatenate(das, axis=0), [], F // DC
        for j in range(nd_):
            js = slice(j * DC, (j + 1) * DC)
            tok = toks(fps[j * FP // nd_], j * FP % nd_, 1, nd_)
            kk = [jnp.tile(pace(jnp.full((8, 128), v, F32), tok), (DC // 8, L // 128))
                  for v in (1.0, 6.0 * GC0 * GC1)]
            uj, hj = u[js], hp[js]
            du.append(da[js] * (hj + (uj * kk[1] * uj + 2.0 * GC0) * ((kk[0] - hj) * hj * uj)))
        du = jnp.concatenate(du, axis=0)
        dsum = (du[:, 0:128] + du[:, 128:256]) + (du[:, 256:384] + du[:, 384:512])
        if it == 0:
            db1_acc[0:F, :] = dsum
            db1_acc[F:F + 64, :] = jnp.zeros((64, 128), F32)
        else:
            db1_acc[0:F, :] += dsum
        dub = du.astype(BF)
        dh2 = _dot(dub, w1T_v[...], _TN)
        fil = _dot(dub, h2)
        wacc(dw1T_acc, w1T_v, ..., fil)

        def ln_bwd_stats(dh, xh, c1, k0, k1):
            p = dh * xh
            vacc(k0, dh)
            vacc(k1, p)
            return rmean(dh * c1), rmean(p * c1)

        ms, dy = [], []
        for c in range(NC):
            dhc = dh2[c * RC:(c + 1) * RC]
            put(x2buf[c], dhc, RC)
            xh = (get(x2buf[c], 4) - wide(pace(mu2[c], toks(fil, 16 * c, 16, 140)))) * wide(rs2[c])
            ms.append(ln_bwd_stats(dhc, xh, 1.0 + cb, 3, 4))
        for c in range(NC):
            xh = (get(x2buf[c], 5) - wide(pace(mu2[c], toks(fil, 64 + 16 * c, 16, 140)))) * wide(rs2[c])
            dx2 = getb(go_v, s * L + c * RC, 2) + wide(rs2[c]) * (
                get(x2buf[c], 1, RC) * (1.0 + cb) - wide(ms[c][0]) - xh * wide(ms[c][1]))
            put(dx2buf[c], dx2)
            vacc(2, dx2 * get(ybuf[c], 1))
            dy.append((dx2 * ga).astype(BF))
        dy = jnp.concatenate(dy, axis=0)
        doT_v[...] = _dot(wo_v[...], dy, _NT).reshape(G, GR, L)
        wacc(dwo_acc, wo_v, ..., _dot(oT, dy))

        def dw2_part(k):
            fs = slice(WSPLIT[k], WSPLIT[k + 1])
            val = _dot(a[fs, :], dfb)
            wacc(dw2_acc, w2_v, (fs, slice(None)), val)
            return val

        def attn_bwd(gi, c2):
            zq = jnp.zeros((64 - GR // 2 - 8, HG * QB), U32)
            steps = [(u, i, j) for u in range(GUB) for i, j in BORDER]
            nper = len(steps) // GUB
            eb, rd, dps, dss, dq, dk, dv, mem = {}, {}, {}, {}, {}, {}, {}, {}

            def gidx(u):
                return u if GUB == G else gi * GUB + u

            seq, mop, rd2 = [], {}, {}
            cover = ((0, 1) if s < NSEG - 1 else ()) + ((2, 3) if s > 0 else ())

            def lhs(xp, h):
                if CHAIN and len(seq) >= CHAIN:
                    tk = [pltpu.bitcast(x, U32) for x in seq[-CHAIN]]
                    if h is None:
                        tok = jnp.concatenate([tk[0] | tk[1], tk[2], tk[3]], axis=0)
                    else:
                        tok = tk[h]
                    xp = jnp.concatenate([xp[0:8], jnp.where(ztrue, xp[8:], tok)], axis=0)
                return _upk(xp)

            def win(xp, h, c):
                return lhs(xp[8 * h:8 * h + 16, c * QB:(c + 1) * QB], h)

            def prep(u):
                g = gidx(u)
                doT = doT_v[g]
                adot = adot_v[g]
                gt = jnp.concatenate([gate_v[g]] * NJ, axis=1)
                dgp = doT * ((amem_v[g] - adot) if s > 0 else -adot)
                dgp = (dgp[:, 0:128] + dgp[:, 128:256]) + (dgp[:, 256:384] + dgp[:, 384:512])
                dg_acc[g] = dgp if it == 0 else dg_acc[g] + dgp
                e = doT * (1.0 - gt) * linv_v[g]
                eb[u] = _pk(e.astype(BF))
                es = e * SCALE
                esp = _pk(es.astype(BF))
                tails = []
                for dl in _segsum(es * adot):
                    hi = dl.astype(BF).astype(F32)
                    tl = jnp.where(prow16 == 0, -hi, jnp.where(prow16 == 1, hi - dl, 0.0))
                    tails.append(_pk(tl.astype(BF)))
                for j in range(NJ):
                    js = slice(j * QB, (j + 1) * QB)
                    top = [jnp.where(prow40 == h, esp[:, js], jnp.uint32(0)) for h in range(HG)]
                    mid = jnp.concatenate([tl[:, js] for tl in tails], axis=1)
                    rd[u, j] = _upk(jnp.concatenate([jnp.concatenate(top, axis=1), mid, zq], axis=0))
                    if j in cover:
                        er = pltpu.roll(esp[:, js], HB, 1)
                        rd2[u, j] = [_upk(jnp.concatenate(
                            [jnp.where(lo40, jnp.where(prow40 == 2 * p, er, jnp.uint32(0)), top[2 * p + 1]),
                             jnp.where(lo8, pltpu.roll(tails[2 * p][:, js], HB, 1), tails[2 * p + 1][:, js]),
                             zq[:, 0:QB]], axis=0)) for p in range(HG // 2)]

            def mem_ops(u):
                g = gidx(u)
                if s < NSEG - 1:
                    kT = _upk(qkvT_v[sd, G + g]).astype(F32)
                    ek = jnp.exp(kT)
                    mop['pk'] = _pk(jnp.where(kT > 0, kT + 1.0, ek).astype(BF))
                    mop['dk'] = jnp.where(kT > 0, 1.0, ek)
                if s > 0:
                    qT = _upk(qkvT_v[sd, g]).astype(F32)
                    eq = jnp.exp(qT)
                    mop['pq'] = _pk(jnp.where(qT > 0, qT + 1.0, eq).astype(BF))
                    mop['dq'] = jnp.where(qT > 0, 1.0, eq)
                    gt = jnp.concatenate([gate_v[g]] * NJ, axis=1)
                    dnum = doT_v[g] * gt * dinv_v[g]
                    dd = _segsum(dnum * amem_v[g])
                    tl = jnp.zeros((16, L), F32)
                    for h in range(HG):
                        tl = jnp.where(prow16 == h, -dd[h], tl)
                    mop['stk'] = _pk(jnp.concatenate([dnum, tl], axis=0).astype(BF))

            def memory(u, k):
                g = gidx(u)

                def wts(xp):
                    if len(seq) >= 4:
                        tok = pltpu.bitcast(jnp.concatenate(seq[-4], axis=1), U32)
                        xp = jnp.concatenate([xp[0:8], jnp.where(ztrue, xp[8:16], tok), xp[16:]], axis=0)
                    return _upk(xp)

                if k == 0:
                    va = jnp.concatenate([qkvT_v[sd, 2 * G + g], jnp.full((8, L), ONES2, U32)], axis=0)
                    r = _dot(dmem_v[g].astype(BF), wts(va), _TN)
                    mem[u, 1] = r * mop['dk']
                elif k == 1:
                    r = mem[u, 2] = _dot(dmem_v[g, 0:GR].astype(BF), wts(mop['pk']))
                elif k == 2:
                    r = _dot(mem_v[sd - 1, g], wts(mop['stk']), _TN)
                    mem[u, 0] = r * mop['dq']
                else:
                    r = _dot(_upk(mop['stk']), wts(mop['pq']), _NT)
                    dmi = jnp.where(bd_mask, r, 0.0)
                    dmem_v[g] = dmi if it == 0 else dmem_v[g] + dmi
                    r = jnp.concatenate([r[0:8], jnp.zeros((8, 128 - GR), F32)] * HG, axis=1)
                seq.append([r[0:8, h * QB:(h + 1) * QB] for h in range(HG)])

            def ptile(g, i, j, h):
                return pT_v[g, _tri(i, j), :, h * QB:(h + 1) * QB]

            def accum(d, key, r):
                seq.append([x[0:8] for x in r])
                d[key] = r if key not in d else [x + y for x, y in zip(d[key], r)]

            def dp_half(t, half):
                u, i, j = steps[t]
                r0 = i * (QB // 2) + half * (QB // 4)
                vp = kvn_v[sd, G + gidx(u), r0:r0 + QB // 4, :]
                if half == 1 and i == j and j in cover:
                    r = [_dot(lhs(vp[h % 2 * 16:h % 2 * 16 + 16], h), rd2[u, j][h // 2]) for h in range(HG)]
                    seq.append([x[0:8] for x in r])
                    d2 = [jnp.concatenate(r[2 * p:2 * p + 2], axis=0) for p in range(HG // 2)]
                    dps[t, half] = jnp.concatenate(
                        [pltpu.roll(d2[0], HB, 1), d2[0], pltpu.roll(d2[1], HB, 1), d2[1]], axis=1)
                    memory(u, j)
                    return
                dps[t, half] = _dot(lhs(vp, None), rd[u, j])
                seq.append([dps[t, half][0:8, h * QB:(h + 1) * QB] for h in range(HG)])

            def dv_step(t):
                u, i, j = steps[t]
                accum(dv, (u, i), [_dot(win(eb[u], h, j), _upk(ptile(gidx(u), i, j, h)), _NT) for h in range(HG)])

            def ds_step(t):
                u, i, j = steps[t]
                dp0, dp1 = _pairs(jnp.concatenate([dps.pop((t, 0)), dps.pop((t, 1))], axis=0))
                dss[t] = []
                for h in range(HG):
                    hs = slice(h * QB, (h + 1) * QB)
                    pt = ptile(gidx(u), i, j, h)
                    dss[t].append(_upk(_ipk(_iupk(pt, 0) * dp0[:, hs], _iupk(pt, 1) * dp1[:, hs])))

            def qk_step(t):
                u, i, j = steps[t]
                g = gidx(u)
                ds = dss.pop(t)
                qTb = qkvT_v[sd, g, :, j * QB:(j + 1) * QB]
                kTb = qkvT_v[sd, G + g, :, i * QB:(i + 1) * QB]
                accum(dk, (u, i), [_dot(win(qTb, h, 0), ds[h], _NT) for h in range(HG)])
                accum(dq, (u, j), [_dot(win(kTb, h, 0), ds[h]) for h in range(HG)])
                if t % nper == nper - 1:
                    for k, d in enumerate((dq, dk, dv)):
                        full = jnp.concatenate([_assemble(d.pop((u, c))) for c in range(NJ)], axis=1)
                        if (u, k) in mem:
                            full = full + mem.pop((u, k))
                        dqkvT_v[s, k * G + g] = _pk(full.astype(BF))

            n = len(steps)
            prep(0)
            for t in range(n + LAG_Q):
                if t < n and t % nper == 0:
                    mem_ops(t // nper)
                if t < n:
                    dp_half(t, 0)
                    dv_step(t)
                    dp_half(t, 1)
                if t == n - 1:
                    dw2_part(0)
                if 0 <= t - LAG_Q < n:
                    qk_step(t - LAG_Q)
                if 0 <= t - 1 < n:
                    ds_step(t - 1)
                if t < n and t % nper == 6 and t // nper + 1 < GUB:
                    prep(t // nper + 1)
            return c2

        if it == NSEG - 1:
            emit(w1T_v, dw1T_hbm, 3)
            emit(wo_v, dwo_hbm, 4)
        attn_bwd(0, 0)
        fil = dw2_part(1)
        if s > 0:
            for k in range(L // 32):
                df_rows(s - 1, k, toks(fil, k, 1, L // 32))
        if s > 1:
            for g in range(G):
                tok = pltpu.bitcast(toks(fil, g, 1, G), U32)
                tok = jnp.concatenate([jnp.concatenate([tok] * NJ, axis=1)] * (GR // 16), axis=0)
                mem_read(s - 1, g, _upk(jnp.where(ztrue, qkvT_v[sd - 1, g], tok)))

        dqkvT = _upk(dqkvT_v[s].reshape(3 * D // 2, L))
        dh1 = _dot(wqkv_v[...], dqkvT).T
        fil = dw2_part(2)
        ms = []
        for c in range(NC):
            cs = slice(c * RC, (c + 1) * RC)
            put(x2buf[c], dh1[cs], RC)
            xh = (getb(x_v, s * L + c * RC, 2) - wide(pace(mu1[s, c], toks(fil, 16 * c, 16, 140)))) * wide(rs1[s, c])
            ms.append(ln_bwd_stats(dh1[cs], xh, 1.0 + ca, 0, 1))
        for c in range(NC):
            cs = slice(c * RC, (c + 1) * RC)
            xh = (getb(x_v, s * L + c * RC, 3) - wide(pace(mu1[s, c], toks(fil, 64 + 16 * c, 16, 140)))) * wide(rs1[s, c])
            dx = get(dx2buf[c], 1) + wide(rs1[s, c]) * (
                get(x2buf[c], 2, RC) * (1.0 + ca) - wide(ms[c][0]) - xh * wide(ms[c][1]))
            go_v[s * L + c * RC:s * L + (c + 1) * RC, :] = dx.astype(BF)
        out_copy(s).start()
        dx_copy(s).start()
        if s > 1:
            cps[15 - s].wait()
        elif s == 1:
            out_copy(3).wait()
        return carry

    for it in range(NSEG):
        phase2(it, 0)

    parts = []

    def dw_qkv(i, r0, r1, dst, k):
        acc = None
        for s in range(NSEG):
            dT = _upk(dqkvT_v[s, i * G:(i + 1) * G].reshape(D // 2, L))
            r = _dot(_upk(h1T_v[s, r0 // 2:r1 // 2, :]), dT, _NT)
            parts.append(r)
            acc = r if acc is None else acc + r
        wqkvT_v[i * D + r0:i * D + r1, :] = acc.astype(BF)
        emit(wqkvT_v.at[i * D + r0:i * D + r1, :], dst.at[r0:r1, :], k)

    emit(w2_v, dw2_hbm, 2)
    vsum = {k: jnp.sum(v, axis=0, keepdims=True) for k, v in vac.items()}
    dw_qkv(0, 0, D, dwq_hbm, 5)
    dmod = jnp.broadcast_to(jnp.concatenate([vsum[k] for k in range(6)], axis=1), (8, 6 * D))
    dw_qkv(1, 0, D, dwk_hbm, 6)
    sacc = []
    for k in range(D // 16):
        rs = slice(k * 16, (k + 1) * 16)
        tok = toks(parts[k // 5], k % 5 * 2 * EP, 2 * EP, 10 * EP)
        sb_ = jnp.concatenate([t for p in range(EP) for t in
                               [pace(silb_v[rs, :], tok[16 * p:16 * p + 8])] * (6 * D // 128 // EP)], axis=1)
        dwm_o[rs, :] = (sb_ * jnp.concatenate([dmod] * 2, axis=0)).astype(BF)
        dm = jnp.where(ztrue, dmod, jnp.concatenate(
            [t for p in range(EP) for t in [tok[16 * p + 8:16 * p + 16]] * (6 * D // 128 // EP)], axis=1))
        r = wm_v[rs, :].astype(F32) * jnp.concatenate([dm] * 2, axis=0)
        rsum = r[:, 0:128]
        for t in range(1, 6 * D // 128):
            rsum = rsum + r[:, t * 128:(t + 1) * 128]
        sacc.append(rsum)
    sacc = jnp.concatenate(sacc, axis=0)
    dsilu = jnp.sum(sacc.T, axis=0, keepdims=True)
    c_v[...] = (dsilu * (sig_c * (1.0 + cf * (1.0 - sig_c)))).astype(BF)
    b1_v[...] = jnp.sum(db1_acc[...].T, axis=0, keepdims=True)[:, 0:F].reshape(F).astype(BF)
    b2_v[...] = vsum['b2'].reshape(D).astype(BF)
    dg_col = jnp.sum(dg_acc[...].reshape(D, 128), axis=1, keepdims=True)
    dg_row = jnp.sum(jnp.where(onehot, dg_col, 0.0), axis=0, keepdims=True)
    beta_v[...] = (dg_row * gate_row * (1.0 - gate_row)).reshape(H).astype(BF)
    for k, (a, b) in enumerate(((c_v, dc_hbm), (beta_v, dbeta_hbm), (b1_v, db1_hbm), (b2_v, db2_hbm))):
        emit(a, b, 16 + k)
    emit(dwm_o, dwm_hbm, 0)
    out_copy(1).wait()
    dw_qkv(2, 0, 512, dwv_hbm, 7)
    dx_copy(1).wait()
    dw_qkv(2, 512, D, dwv_hbm, 1)

    for s in (0, 2, 3):
        if s < 3:
            out_copy(s).wait()
        dx_copy(s).wait()
    for cp in fin:
        cp.wait()


@jax.jit
def pallas_adaLN_cond__memory_aug_infini_attn__dense_activation_gelu__prompt_kernel(
    A_x: jax.Array,
    A_wq: jax.Array,
    A_wk: jax.Array,
    A_wv: jax.Array,
    A_wo: jax.Array,
    A_beta: jax.Array,
    B_x: jax.Array,
    B_w1: jax.Array,
    B_b1: jax.Array,
    B_w2: jax.Array,
    B_b2: jax.Array,
    c: jax.Array,
    w_mod: jax.Array,
    grad_out: jax.Array,
):
    any_spec = pl.BlockSpec(memory_space=pltpu.MemorySpace.HBM)
    sds = jax.ShapeDtypeStruct
    V = pltpu.VMEM
    out_shape = (
        sds((S, D), BF), sds((S, D), BF),
        sds((D, D), BF), sds((D, D), BF), sds((D, D), BF), sds((D, D), BF),
        sds((H,), BF),
        sds((F, D), BF), sds((F,), BF), sds((F, D), BF), sds((D,), BF),
        sds((1, D), BF), sds((D, 6 * D), BF),
    )
    out_specs = (any_spec,) * 13
    scratch = [
        V((H,), BF), V((F,), BF), V((D,), BF), V((1, D), BF), V((F, 128), F32), V((1, D), F32),
        V((S, D), BF), V((S, D), BF), V((D, 3 * D), BF), V((3 * D, D), BF), V((D, D), BF),
        V((F, D), BF), V((F, D), BF), V((D, 6 * D), BF),
        V((8, 6 * D), F32), V((G, GR, 128), F32), V((NSEG, D // 2, L), U32),
        V((NSEG, 4 * G, GR // 2, L), U32), V((NSEG, 2 * G, L // 2, 128), U32),
        V((NSEG - 1, G, MR, GR), BF), V((G, MR, GR), F32),
        V((G, NJ * (NJ + 1) // 2, QB // 2, HG * QB), U32),
        V((G, GR, L), F32), V((G, GR, L), F32), V((G, GR, L), F32), V((G, GR, L), F32),
        V((G, GR // 2, L), U32), V((G, GR, L), F32), V((NSEG, 3 * G, GR // 2, L), U32),
        V((S, D), BF),
        V((D, D), F32), V((F, D), F32), V((F, D), F32),
        V((D, 128), F32), V((G, GR, 128), F32),
        V((D, 6 * D), BF), V((3, G, GR // 2, D), U32), V((F + 64, 128), F32),
        V((8, 128), jnp.int32), pltpu.SMEM((8, 128), jnp.int32), pltpu.SMEM((NZ,), jnp.int32),
        pltpu.SemaphoreType.DMA((20,)), pltpu.SemaphoreType.DMA((20,)),
    ] + [V((2, QB, HG * QB), F32)] * NSLOT + [V((RC + 8, D), F32)] * (2 * NC) + [V((2 * RC + 8, D), F32)] * NC
    outs = pl.pallas_call(
        _kernel,
        out_shape=out_shape,
        in_specs=[any_spec] * 13,
        out_specs=out_specs,
        scratch_shapes=scratch,
        compiler_params=pltpu.CompilerParams(vmem_limit_bytes=120 * 1024 * 1024),
    )(A_x.reshape(S, D), grad_out.reshape(S, D), A_wq, A_wk, A_wv, A_wo, B_w1.T, B_w2, w_mod,
      A_beta, B_b1, B_b2, c)
    (out, dx, dwq, dwk, dwv, dwo, dbeta, dw1T, db1, dw2, db2, dc, dwm) = outs
    return (out.reshape(1, S, D), dx.reshape(1, S, D), dwq, dwk, dwv, dwo, dbeta,
            dw1T.T, db1, dw2, db2, dc, dwm)
```
